```python
import os as _os
_os.environ.setdefault("JAX_PLATFORMS", "cpu")
import jax
import jax.numpy as jnp

def _softmax(x, axis=-1):
    return jax.nn.softmax(x, axis=axis)
def _gelu(x):
    return jax.nn.gelu(x, approximate=True)
def _silu(x):
    return jax.nn.silu(x)
def _sigmoid(x):
    return jax.nn.sigmoid(x)
def _layernorm(x, axis=-1, eps=1e-5):
    m = jnp.mean(x, axis=axis, keepdims=True)
    v = jnp.var(x, axis=axis, keepdims=True)
    return (x - m) / jnp.sqrt(v + eps)
def _scatter_add(tgt, idx, src, axis=0):
    return tgt.at[idx].add(src)
def _segment_sum(src, seg, n):
    return jax.ops.segment_sum(src, seg, n)
class _Rng:
    def __init__(self, key):
        self._k = key
    def _next(self):
        self._k, sub = jax.random.split(self._k)
        return sub
    def normal(self, shape):
        return jax.random.normal(self._next(), shape, dtype=jnp.bfloat16)
    def randint(self, lo, hi, shape):
        return jax.random.randint(self._next(), shape, lo, hi, dtype=jnp.int32)
    def uniform(self, shape, lo=0.0, hi=1.0):
        return jax.random.uniform(self._next(), shape, jnp.bfloat16, lo, hi)
    def permutation(self, n):
        return jax.random.permutation(self._next(), n)


kernel_name = 'standalone__mha_softmax__near_ridge'

def setup_inputs():
    _rng = _Rng(jax.random.key(int.from_bytes(__import__("os").urandom(4), "little")))
    _w = (lambda a: (lambda t: t.astype(jnp.bfloat16) if jnp.issubdtype(t.dtype, jnp.floating) else t)(jnp.asarray(a)))
    B, H, Sq, Sk, D = 8, 32, 496, 512, 192
    return {
        "q": _w((lambda *s: _rng.normal(s) * 0.05)(B, H, Sq, D)),
        "k": _w((lambda *s: _rng.normal(s) * 3.2)(B, H, Sk, D)),
        "v": _w((lambda *s: _rng.normal(s) * 0.05)(B, H, Sk, D)),
    }

def reference(q, k, v):
    scale = q.shape[-1] ** -0.5
    scores = jnp.einsum("bhqd,bhkd->bhqk", q, k) * scale
    p = _softmax(scores, axis=-1)
    return jnp.einsum("bhqk,bhkd->bhqd", p, v)
```

```python
import functools
import math

import jax
import jax.numpy as jnp
from jax import lax
import jax.experimental.pallas as pl
import jax.experimental.pallas.tpu as pltpu

_U = 8
_RAMP = (1, 1, 2, 4, 4, 4)
_NBUF = 3


def _attention_kernel(q_hbm, k_hbm, v_hbm, o_hbm,
                      q_scr, k_scr, v_scr, o_scr,
                      rq, rk, rv, ro, q0_scr, qt_scr,
                      s00, s01, s10, s11,
                      isem, osem, rsem, rosem, *, n_heads, scale):
    U, ramp, NBUF = _U, _RAMP, _NBUF
    R = sum(ramp)
    NIT = (n_heads - R) // U
    HU = U // 2
    Sq = q_scr.shape[-1]
    Sk = k_scr.shape[-1]
    c = scale * math.log2(math.e)
    q_halves = ((0, 256), (256, Sq))
    k_halves = ((0, Sk // 2), (Sk // 2, Sk))
    s_scr = (s00, s01, s10, s11)

    def in_copies(it, slot):
        h0 = R + it * U
        h_last = jnp.minimum(h0 + U, n_heads - 1)
        return (
            pltpu.make_async_copy(k_hbm.at[pl.ds(h0, U)], k_scr.at[slot], isem.at[slot, 0]),
            pltpu.make_async_copy(q_hbm.at[pl.ds(h0 + 1, U - 1)],
                                  q_scr.at[slot, pl.ds(0, U - 1)], isem.at[slot, 1]),
            pltpu.make_async_copy(q_hbm.at[h_last], q_scr.at[slot, U - 1], isem.at[slot, 2]),
            pltpu.make_async_copy(v_hbm.at[pl.ds(h0, U)], v_scr.at[slot], isem.at[slot, 3]),
        )

    def out_copy(it, slot, half):
        return pltpu.make_async_copy(o_scr.at[slot, pl.ds(half * HU, HU)],
                                     o_hbm.at[pl.ds(R + it * U + half * HU, HU)],
                                     osem.at[slot, half])

    def ramp_copies(i):
        a, n = sum(ramp[:i]), ramp[i]
        return (
            pltpu.make_async_copy(k_hbm.at[pl.ds(a, n)], rk.at[pl.ds(a, n)], rsem.at[i, 0]),
            pltpu.make_async_copy(q_hbm.at[pl.ds(a + 1, n)], rq.at[pl.ds(a, n)], rsem.at[i, 1]),
            pltpu.make_async_copy(v_hbm.at[pl.ds(a, n)], rv.at[pl.ds(a, n)], rsem.at[i, 2]),
        )

    def ramp_out(i):
        a, n = sum(ramp[:i]), ramp[i]
        return pltpu.make_async_copy(ro.at[pl.ds(a, n)], o_hbm.at[pl.ds(a, n)], rosem.at[i])

    q0_copy = pltpu.make_async_copy(q_hbm.at[0], q0_scr, rsem.at[len(ramp), 0])

    def segment(n, q_ref, k_ref, v_ref, o_ref, ia, ib, hooks):
        def qk(g):
            q = qt_scr[...] if g == 0 else q_ref[g - 1].T
            for h, (a, b) in enumerate(k_halves):
                s = jnp.dot(q, k_ref[g, :, a:b], preferred_element_type=jnp.float32)
                s_scr[(g % 2) * 2 + h][ia] = s

        def softmax(g, a, b):
            s = jnp.concatenate([s_scr[(g % 2) * 2 + 0][ib, a:b],
                                 s_scr[(g % 2) * 2 + 1][ib, a:b]], axis=1)
            m = jnp.max(s, axis=1, keepdims=True)
            p = jnp.exp2((s - m) * c)
            l = jnp.sum(p, axis=1, keepdims=True)
            r = pl.reciprocal(l, approx=True)
            r = r * (2.0 - l * r)
            return (p * r).astype(jnp.bfloat16)

        def pv(g, ps):
            vt = v_ref[g]
            for (a, b), p in zip(q_halves, ps):
                ot = lax.dot_general(vt, p, (((1,), (1,)), ((), ())),
                                     preferred_element_type=jnp.float32)
                o_ref[g, :, a:b] = ot.astype(o_ref.dtype)

        qk(0)
        for g in range(n):
            if g + 1 < n:
                qk(g + 1)
            else:
                qt_scr[...] = q_ref[n - 1].T
            pv(g, [softmax(g, a, b) for a, b in q_halves])
            if g in hooks:
                hooks[g]()

    def start_all(copies):
        for cp in copies:
            cp.start()

    issue = [functools.partial(lambda i: start_all(ramp_copies(i)), i) for i in range(len(ramp))]
    issue += [functools.partial(lambda j: start_all(in_copies(j, j)), j) for j in range(NBUF - 1)]
    issued = [0]

    def issue_upto(n):
        while issued[0] < min(n, len(issue)):
            issue[issued[0]]()
            issued[0] += 1

    q0_copy.start()
    issue_upto(2)
    q0_copy.wait()
    qt_scr[...] = q0_scr[...].T
    for i, n in enumerate(ramp):
        a = sum(ramp[:i])
        for cp in ramp_copies(i):
            cp.wait()
        issue_upto(i + 3)
        segment(n, rq.at[pl.ds(a, n)], rk.at[pl.ds(a, n)], rv.at[pl.ds(a, n)],
                ro.at[pl.ds(a, n)], 0, 0, {})
        ramp_out(i).start()
    issue_upto(len(issue))

    def body(it, zero):
        slot = lax.rem(it, NBUF)
        oslot = lax.rem(it, 2)

        @pl.when(it + (NBUF - 1) < NIT)
        def _():
            start_all(in_copies(it + (NBUF - 1), lax.rem(it + (NBUF - 1), NBUF)))

        @pl.when(it >= 2)
        def _():
            out_copy(it - 2, oslot, 0).wait()
            out_copy(it - 2, oslot, 1).wait()

        for cp in in_copies(it, slot):
            cp.wait()

        segment(U, q_scr.at[slot], k_scr.at[slot], v_scr.at[slot], o_scr.at[oslot],
                it // NIT, zero, {HU - 1: lambda: out_copy(it, oslot, 0).start()})
        out_copy(it, oslot, 1).start()
        return zero

    lax.fori_loop(0, NIT, body, 0)

    for it in (NIT - 2, NIT - 1):
        out_copy(it, it % 2, 0).wait()
        out_copy(it, it % 2, 1).wait()
    for i in range(len(ramp)):
        ramp_out(i).wait()


@jax.jit
def pallas_standalone__mha_softmax__near_ridge_kernel(
    q: jax.Array,
    k: jax.Array,
    v: jax.Array,
):
    B, H, Sq, D = q.shape
    Sk = k.shape[2]
    n_heads = B * H
    U, ramp, NBUF = _U, _RAMP, _NBUF
    R = sum(ramp)
    assert (n_heads - R) % U == 0 and (n_heads - R) // U >= 2
    assert Sk % 256 == 0 and 256 < Sq <= 512

    qt = jnp.swapaxes(q, 2, 3).reshape(n_heads, D, Sq)
    kt = jnp.swapaxes(k, 2, 3).reshape(n_heads, D, Sk)
    vt = jnp.swapaxes(v, 2, 3).reshape(n_heads, D, Sk)

    dt = q.dtype
    scratch = [
        pltpu.VMEM((NBUF, U, D, Sq), dt), pltpu.VMEM((NBUF, U, D, Sk), dt),
        pltpu.VMEM((NBUF, U, D, Sk), dt), pltpu.VMEM((2, U, D, Sq), dt),
        pltpu.VMEM((R, D, Sq), dt), pltpu.VMEM((R, D, Sk), dt),
        pltpu.VMEM((R, D, Sk), dt), pltpu.VMEM((R, D, Sq), dt),
        pltpu.VMEM((D, Sq), dt), pltpu.VMEM((Sq, D), dt),
    ]
    scratch += [pltpu.VMEM((1, Sq, Sk // 2), jnp.float32) for _ in range(4)]
    scratch += [
        pltpu.SemaphoreType.DMA((NBUF, 4)), pltpu.SemaphoreType.DMA((2, 2)),
        pltpu.SemaphoreType.DMA((len(ramp) + 1, 3)), pltpu.SemaphoreType.DMA((len(ramp),)),
    ]

    ot = pl.pallas_call(
        functools.partial(_attention_kernel, n_heads=n_heads, scale=D ** -0.5),
        in_specs=[pl.BlockSpec(memory_space=pl.ANY)] * 3,
        out_specs=pl.BlockSpec(memory_space=pl.ANY),
        out_shape=jax.ShapeDtypeStruct((n_heads, D, Sq), dt),
        scratch_shapes=scratch,
        compiler_params=pltpu.CompilerParams(
            vmem_limit_bytes=64 * 1024 * 1024, disable_bounds_checks=True),
    )(qt, kt, vt)
    return jnp.swapaxes(ot.reshape(B, H, D, Sq), 2, 3)
```

```python
import functools
import math

import jax
import jax.numpy as jnp
from jax import lax
import jax.experimental.pallas as pl
import jax.experimental.pallas.tpu as pltpu

_RAMP = (1, 1, 2, 3)
_UA, _NA = 4, 6
_U = 16
_NBUF = 3
_NOUT = 3
_NO = 4


def _attention_kernel(q_hbm, k_hbm, v_hbm, o_hbm,
                      q_scr, k_scr, v_scr, o_scr,
                      rq, rk, rv, ro,
                      q01, k0, e_v, e_o, qt_scr,
                      s00, s01, s10, s11,
                      isem, osem, rsem, asem, xsem, psem, *, n_heads, scale):
    ramp, UA, NA, U, NBUF, NOUT, NO = _RAMP, _UA, _NA, _U, _NBUF, _NOUT, _NO
    R0 = sum(ramp)
    R = R0 + UA * NA
    NIT = (n_heads - 1 - R) // U
    HU = U // NO
    last = n_heads - 1
    Sq = q_scr.shape[-1]
    Sk = k_scr.shape[-1]
    c = scale * math.log2(math.e)
    q_halves = ((0, 256), (256, Sq))
    k_halves = ((0, Sk // 2), (Sk // 2, Sk))
    s_scr = (s00, s01, s10, s11)
    copy = pltpu.make_async_copy

    def in_copies(it, slot):
        a = R + it * U
        return (
            copy(k_hbm.at[pl.ds(a + 1, U)], k_scr.at[slot], isem.at[slot, 0]),
            copy(v_hbm.at[pl.ds(a, U)], v_scr.at[slot], isem.at[slot, 1]),
            copy(q_hbm.at[pl.ds(a + 2, U - 1)], q_scr.at[slot, pl.ds(0, U - 1)], isem.at[slot, 2]),
            copy(q_hbm.at[jnp.minimum(a + U + 1, last)], q_scr.at[slot, U - 1], isem.at[slot, 3]),
        )

    def out_copy(it, slot, j):
        return copy(o_scr.at[slot, pl.ds(j * HU, HU)],
                    o_hbm.at[pl.ds(R + it * U + j * HU, HU)], osem.at[slot, j])

    def start_copies(a, n, sem):
        return (
            copy(k_hbm.at[pl.ds(a + 1, n)], rk.at[pl.ds(a, n)], sem.at[0]),
            copy(v_hbm.at[pl.ds(a, n)], rv.at[pl.ds(a, n)], sem.at[1]),
            copy(q_hbm.at[pl.ds(a + 2, n)], rq.at[pl.ds(a, n)], sem.at[2]),
        )

    def start_out(a, n, sem):
        return copy(ro.at[pl.ds(a, n)], o_hbm.at[pl.ds(a, n)], sem.at[3])

    def ramp_copies(i):
        return start_copies(sum(ramp[:i]), ramp[i], rsem.at[i])

    def ramp_out(i):
        return start_out(sum(ramp[:i]), ramp[i], rsem.at[i])

    def a_copies(i):
        return start_copies(R0 + i * UA, UA, asem.at[i])

    def a_out(i):
        return start_out(R0 + i * UA, UA, asem.at[i])

    k0_copy = copy(k_hbm.at[0], k0, xsem.at[0])
    q01_copy = copy(q_hbm.at[pl.ds(0, 2)], q01, xsem.at[1])
    ev_copy = copy(v_hbm.at[last], e_v, xsem.at[2])
    eo_copy = copy(e_o, o_hbm.at[last], xsem.at[3])

    def qk(q, kt_ref, par, ia):
        for h, (a, b) in enumerate(k_halves):
            s = jnp.dot(q, kt_ref[:, a:b], preferred_element_type=jnp.float32)
            s_scr[par * 2 + h][ia] = s

    def softmax(par, a, b, ib):
        s0 = s_scr[par * 2 + 0][ib, a:b]
        s1 = s_scr[par * 2 + 1][ib, a:b]
        m = jnp.maximum(jnp.max(s0, axis=1, keepdims=True), jnp.max(s1, axis=1, keepdims=True))
        p0 = jnp.exp2((s0 - m) * c)
        p1 = jnp.exp2((s1 - m) * c)
        l = jnp.sum(p0, axis=1, keepdims=True) + jnp.sum(p1, axis=1, keepdims=True)
        r = pl.reciprocal(l, approx=True)
        r = r * (2.0 - l * r)
        return jnp.concatenate([(p0 * r).astype(jnp.bfloat16),
                                (p1 * r).astype(jnp.bfloat16)], axis=1)

    def pv(vt_ref, o_ref, par, ib):
        ps = [softmax(par, a, b, ib) for a, b in q_halves]
        vt = vt_ref[...]
        for (a, b), p in zip(q_halves, ps):
            ot = lax.dot_general(vt, p, (((1,), (1,)), ((), ())),
                                 preferred_element_type=jnp.float32)
            o_ref[:, a:b] = ot.astype(o_ref.dtype)

    def segment(n, par0, q_ref, k_ref, v_ref, o_ref, ia, ib, hooks):
        for g in range(n):
            q = qt_scr[...] if g == 0 else q_ref[g - 1].T
            qk(q, k_ref.at[g], (par0 + g + 1) % 2, ia)
            if g == n - 1:
                qt_scr[...] = q_ref[n - 1].T
            pv(v_ref.at[g], o_ref.at[g], (par0 + g) % 2, ib)
            if g in hooks:
                hooks[g]()

    def start_all(copies):
        for cp in copies:
            cp.start()

    groups = [(k0_copy,), (q01_copy,)]
    groups += [ramp_copies(i) for i in range(len(ramp))]
    groups += [a_copies(i) for i in range(NA)]
    groups += [in_copies(j, j) for j in range(NBUF - 1)]
    groups += [(ev_copy,)]
    for grp in groups:
        start_all(grp)
        pl.semaphore_signal(psem, 1)
        pl.semaphore_wait(psem, 1)

    k0_copy.wait()
    q01_copy.wait()
    qk(q01[0].T, k0, 0, 0)
    qt_scr[...] = q01[1].T
    for i, n in enumerate(ramp):
        a = sum(ramp[:i])
        for cp in ramp_copies(i):
            cp.wait()
        segment(n, a % 2, rq.at[pl.ds(a, n)], rk.at[pl.ds(a, n)], rv.at[pl.ds(a, n)],
                ro.at[pl.ds(a, n)], 0, 0, {})

    def body_a(i, zero):
        for cp in a_copies(i):
            cp.wait()
        a = R0 + i * UA
        segment(UA, R0 % 2, rq.at[pl.ds(a, UA)], rk.at[pl.ds(a, UA)], rv.at[pl.ds(a, UA)],
                ro.at[pl.ds(a, UA)], i // NA, zero, {})
        return zero

    lax.fori_loop(0, NA, body_a, 0)

    def body(it, zero):
        slot = lax.rem(it, NBUF)
        oslot = lax.rem(it, NOUT)

        @pl.when(it + (NBUF - 1) < NIT)
        def _():
            start_all(in_copies(it + (NBUF - 1), lax.rem(it + (NBUF - 1), NBUF)))

        @pl.when(it < NA)
        def _():
            a_out(it).start()

        @pl.when(it == NA)
        def _():
            for i in range(len(ramp)):
                ramp_out(i).start()

        @pl.when(it >= NOUT)
        def _():
            for j in range(NO):
                out_copy(it - NOUT, oslot, j).wait()

        for cp in in_copies(it, slot):
            cp.wait()

        hooks = {HU * (j + 1) - 1: functools.partial(lambda j: out_copy(it, oslot, j).start(), j)
                 for j in range(NO)}
        segment(U, R % 2, q_scr.at[slot], k_scr.at[slot], v_scr.at[slot], o_scr.at[oslot],
                it // NIT, zero, hooks)
        return zero

    lax.fori_loop(0, NIT, body, 0)

    ev_copy.wait()
    pv(e_v, e_o, last % 2, 0)
    eo_copy.start()
    for it in range(NIT - NOUT, NIT):
        for j in range(NO):
            out_copy(it, it % NOUT, j).wait()
    for i in range(len(ramp)):
        ramp_out(i).wait()
    for i in range(NA):
        a_out(i).wait()
    eo_copy.wait()


@jax.jit
def pallas_standalone__mha_softmax__near_ridge_kernel(
    q: jax.Array,
    k: jax.Array,
    v: jax.Array,
):
    B, H, Sq, D = q.shape
    Sk = k.shape[2]
    n_heads = B * H
    ramp, UA, NA, U, NBUF, NOUT, NO = _RAMP, _UA, _NA, _U, _NBUF, _NOUT, _NO
    R = sum(ramp) + UA * NA
    NIT = (n_heads - 1 - R) // U
    assert R + NIT * U + 1 == n_heads and NIT > max(NA, NOUT) and NIT >= NBUF
    assert U % 2 == 0 and UA % 2 == 0 and U % NO == 0
    assert Sk % 256 == 0 and 256 < Sq <= 512

    qt = jnp.swapaxes(q, 2, 3).reshape(n_heads, D, Sq)
    kt = jnp.swapaxes(k, 2, 3).reshape(n_heads, D, Sk)
    vt = jnp.swapaxes(v, 2, 3).reshape(n_heads, D, Sk)

    dt = q.dtype
    vmem, dma = pltpu.VMEM, pltpu.SemaphoreType.DMA
    scratch = [
        vmem((NBUF, U, D, Sq), dt), vmem((NBUF, U, D, Sk), dt), vmem((NBUF, U, D, Sk), dt),
        vmem((NOUT, U, D, Sq), dt),
        vmem((R, D, Sq), dt), vmem((R, D, Sk), dt), vmem((R, D, Sk), dt), vmem((R, D, Sq), dt),
        vmem((2, D, Sq), dt), vmem((D, Sk), dt), vmem((D, Sk), dt), vmem((D, Sq), dt),
        vmem((Sq, D), dt),
    ]
    scratch += [vmem((1, Sq, Sk // 2), jnp.float32) for _ in range(4)]
    scratch += [
        dma((NBUF, 4)), dma((NOUT, NO)), dma((len(ramp), 4)), dma((NA, 4)), dma((4,)),
        pltpu.SemaphoreType.REGULAR,
    ]

    ot = pl.pallas_call(
        functools.partial(_attention_kernel, n_heads=n_heads, scale=D ** -0.5),
        in_specs=[pl.BlockSpec(memory_space=pl.ANY)] * 3,
        out_specs=pl.BlockSpec(memory_space=pl.ANY),
        out_shape=jax.ShapeDtypeStruct((n_heads, D, Sq), dt),
        scratch_shapes=scratch,
        compiler_params=pltpu.CompilerParams(
            vmem_limit_bytes=100 * 1024 * 1024, disable_bounds_checks=True),
    )(qt, kt, vt)
    return jnp.swapaxes(ot.reshape(B, H, D, Sq), 2, 3)
```

```python
import functools
import math

import jax
import jax.numpy as jnp
from jax import lax
import jax.experimental.pallas as pl
import jax.experimental.pallas.tpu as pltpu

_RAMP = (1, 1, 2, 2)
_UA, _NA = 4, 6
_U = 16
_NBUF = 3
_NOUT = 2
_NO = 4


def _attention_kernel(q_hbm, k_hbm, v_hbm, o_hbm,
                      q_scr, k_scr, v_scr, o_scr,
                      rq, rk, rv, ro,
                      q01, k0, e_k, e_v, e_o, qt_scr,
                      s00, s01, s10, s11,
                      isem, osem, rsem, asem, xsem, lsem, psem, *, n_heads, scale):
    ramp, UA, NA, U, NBUF, NOUT, NO = _RAMP, _UA, _NA, _U, _NBUF, _NOUT, _NO
    R0 = sum(ramp)
    R = R0 + UA * NA
    NIT = (n_heads - 2 - R) // U
    HU = U // NO
    last = n_heads - 1
    Sq = q_scr.shape[-1]
    Sk = k_scr.shape[-1]
    c = scale * math.log2(math.e)
    q_halves = ((0, 256), (256, Sq))
    k_halves = ((0, Sk // 2), (Sk // 2, Sk))
    s_scr = (s00, s01, s10, s11)
    copy = pltpu.make_async_copy

    def in_copies(it, slot):
        a = R + it * U
        return (
            copy(k_hbm.at[pl.ds(a + 1, U)], k_scr.at[slot], isem.at[slot, 0]),
            copy(v_hbm.at[pl.ds(a, U)], v_scr.at[slot], isem.at[slot, 1]),
            copy(q_hbm.at[pl.ds(a + 2, U)], q_scr.at[slot], isem.at[slot, 2]),
        )

    def out_copy(it, slot, j):
        return copy(o_scr.at[slot, pl.ds(j * HU, HU)],
                    o_hbm.at[pl.ds(R + it * U + j * HU, HU)], osem.at[slot])

    def out_wait(slot):
        copy(o_scr.at[slot], o_scr.at[slot], osem.at[slot]).wait()

    def start_copies(a, n, sem):
        return (
            copy(k_hbm.at[pl.ds(a + 1, n)], rk.at[pl.ds(a, n)], sem.at[0]),
            copy(v_hbm.at[pl.ds(a, n)], rv.at[pl.ds(a, n)], sem.at[1]),
            copy(q_hbm.at[pl.ds(a + 2, n)], rq.at[pl.ds(a, n)], sem.at[2]),
        )

    LP = R // NIT

    def late_out(a, n):
        return copy(ro.at[pl.ds(a, n)], o_hbm.at[pl.ds(a, n)], lsem)

    def ramp_copies(i):
        return start_copies(sum(ramp[:i]), ramp[i], rsem.at[i])

    def a_copies(i):
        return start_copies(R0 + i * UA, UA, asem.at[i])

    k0_copy = copy(k_hbm.at[0], k0, xsem.at[0])
    q01_copy = copy(q_hbm.at[pl.ds(0, 2)], q01, xsem.at[1])
    ek_copy = copy(k_hbm.at[pl.ds(last, 1)], e_k, xsem.at[2])
    ev_copy = copy(v_hbm.at[pl.ds(last - 1, 2)], e_v, xsem.at[3])
    eo_copy = copy(e_o, o_hbm.at[pl.ds(last - 1, 2)], xsem.at[4])

    def qk(q, kt_ref, par, ia):
        for h, (a, b) in enumerate(k_halves):
            s = jnp.dot(q, kt_ref[:, a:b], preferred_element_type=jnp.float32)
            s_scr[par * 2 + h][ia] = s

    def softmax(par, a, b, ib):
        s0 = s_scr[par * 2 + 0][ib, a:b]
        s1 = s_scr[par * 2 + 1][ib, a:b]
        m = jnp.maximum(jnp.max(s0, axis=1, keepdims=True), jnp.max(s1, axis=1, keepdims=True))
        p0 = jnp.exp2((s0 - m) * c)
        p1 = jnp.exp2((s1 - m) * c)
        l = jnp.sum(p0, axis=1, keepdims=True) + jnp.sum(p1, axis=1, keepdims=True)
        r = pl.reciprocal(l, approx=True)
        r = r * (2.0 - l * r)
        return jnp.concatenate([(p0 * r).astype(jnp.bfloat16),
                                (p1 * r).astype(jnp.bfloat16)], axis=1)

    def pv(vt_ref, o_ref, par, ib):
        ps = [softmax(par, a, b, ib) for a, b in q_halves]
        vt = vt_ref[...]
        for (a, b), p in zip(q_halves, ps):
            ot = lax.dot_general(vt, p, (((1,), (1,)), ((), ())),
                                 preferred_element_type=jnp.float32)
            o_ref[:, a:b] = ot.astype(o_ref.dtype)

    def segment(n, par0, q_ref, k_ref, v_ref, o_ref, ia, ib, hooks, lookahead=True):
        for g in range(n):
            q = qt_scr[...] if g == 0 else q_ref[g - 1].T
            qk(q, k_ref.at[g], (par0 + g + 1) % 2, ia)
            if g == n - 1 and lookahead:
                qt_scr[...] = q_ref[n - 1].T
            pv(v_ref.at[g], o_ref.at[g], (par0 + g) % 2, ib)
            if g in hooks:
                hooks[g]()

    def start_all(copies):
        for cp in copies:
            cp.start()

    groups = [(k0_copy,), (q01_copy,)]
    groups += [ramp_copies(i) for i in range(len(ramp))]
    groups += [a_copies(i) for i in range(NA)]
    groups += [in_copies(j, j) for j in range(NBUF - 1)]
    groups += [(ek_copy, ev_copy)]
    for grp in groups:
        start_all(grp)
        pl.semaphore_signal(psem, 1)
        pl.semaphore_wait(psem, 1)

    k0_copy.wait()
    q01_copy.wait()
    qk(q01[0].T, k0, 0, 0)
    qt_scr[...] = q01[1].T
    for i, n in enumerate(ramp):
        a = sum(ramp[:i])
        for cp in ramp_copies(i):
            cp.wait()
        segment(n, a % 2, rq.at[pl.ds(a, n)], rk.at[pl.ds(a, n)], rv.at[pl.ds(a, n)],
                ro.at[pl.ds(a, n)], 0, 0, {})

    def body_a(i, zero):
        for cp in a_copies(i):
            cp.wait()
        a = R0 + i * UA
        segment(UA, R0 % 2, rq.at[pl.ds(a, UA)], rk.at[pl.ds(a, UA)], rv.at[pl.ds(a, UA)],
                ro.at[pl.ds(a, UA)], i // NA, zero, {})
        return zero

    lax.fori_loop(0, NA, body_a, 0)

    def body(it, carry):
        zero, slot = carry
        nslot = jnp.where(slot == 0, NBUF - 1, slot - 1)
        oslot = lax.rem(it, NOUT)

        @pl.when(it + (NBUF - 1) < NIT)
        def _():
            start_all(in_copies(it + (NBUF - 1), nslot))

        @pl.when(it >= NOUT)
        def _():
            out_wait(oslot)

        for cp in in_copies(it, slot):
            cp.wait()

        hooks = {HU * (j + 1) - 1: functools.partial(lambda j: out_copy(it, oslot, j).start(), j)
                 for j in range(NO)}
        assert 1 not in hooks
        hooks[1] = lambda: late_out(it * LP, LP).start()
        segment(U, R % 2, q_scr.at[slot], k_scr.at[slot], v_scr.at[slot], o_scr.at[oslot],
                it // NIT, zero, hooks)
        return zero, jnp.where(slot == NBUF - 1, 0, slot + 1)

    lax.fori_loop(0, NIT, body, (jnp.int32(0), jnp.int32(0)))

    if R > LP * NIT:
        late_out(LP * NIT, R - LP * NIT).start()
    ek_copy.wait()
    ev_copy.wait()
    segment(1, last % 2 ^ 1, None, e_k, e_v, e_o, 0, 0, {}, lookahead=False)
    pv(e_v.at[1], e_o.at[1], last % 2, 0)
    eo_copy.start()
    for slot in range(NOUT):
        out_wait(slot)
    late_out(0, R).wait()
    eo_copy.wait()


@jax.jit
def pallas_standalone__mha_softmax__near_ridge_kernel(
    q: jax.Array,
    k: jax.Array,
    v: jax.Array,
):
    B, H, Sq, D = q.shape
    Sk = k.shape[2]
    n_heads = B * H
    ramp, UA, NA, U, NBUF, NOUT, NO = _RAMP, _UA, _NA, _U, _NBUF, _NOUT, _NO
    R = sum(ramp) + UA * NA
    NIT = (n_heads - 2 - R) // U
    assert R + NIT * U + 2 == n_heads and NIT > max(NA, NOUT) and NIT >= NBUF
    assert U % 2 == 0 and UA % 2 == 0 and U % NO == 0
    assert Sk % 256 == 0 and 256 < Sq <= 512

    qt = jnp.swapaxes(q, 2, 3).reshape(n_heads, D, Sq)
    kt = jnp.swapaxes(k, 2, 3).reshape(n_heads, D, Sk)
    vt = jnp.swapaxes(v, 2, 3).reshape(n_heads, D, Sk)

    dt = q.dtype
    vmem, dma = pltpu.VMEM, pltpu.SemaphoreType.DMA
    scratch = [
        vmem((NBUF, U, D, Sq), dt), vmem((NBUF, U, D, Sk), dt), vmem((NBUF, U, D, Sk), dt),
        vmem((NOUT, U, D, Sq), dt),
        vmem((R, D, Sq), dt), vmem((R, D, Sk), dt), vmem((R, D, Sk), dt), vmem((R, D, Sq), dt),
        vmem((2, D, Sq), dt), vmem((D, Sk), dt), vmem((1, D, Sk), dt), vmem((2, D, Sk), dt),
        vmem((2, D, Sq), dt), vmem((Sq, D), dt),
    ]
    scratch += [vmem((1, Sq, Sk // 2), jnp.float32) for _ in range(4)]
    scratch += [
        dma((NBUF, 3)), dma((NOUT,)), dma((len(ramp), 3)), dma((NA, 3)), dma((5,)), dma,
        pltpu.SemaphoreType.REGULAR,
    ]

    ot = pl.pallas_call(
        functools.partial(_attention_kernel, n_heads=n_heads, scale=D ** -0.5),
        in_specs=[pl.BlockSpec(memory_space=pl.ANY)] * 3,
        out_specs=pl.BlockSpec(memory_space=pl.ANY),
        out_shape=jax.ShapeDtypeStruct((n_heads, D, Sq), dt),
        scratch_shapes=scratch,
        compiler_params=pltpu.CompilerParams(
            vmem_limit_bytes=100 * 1024 * 1024,
            disable_bounds_checks=True,
            disable_semaphore_checks=True),
    )(qt, kt, vt)
    return jnp.swapaxes(ot.reshape(B, H, D, Sq), 2, 3)
```

```python
import functools
import math

import jax
import jax.numpy as jnp
from jax import lax
import jax.experimental.pallas as pl
import jax.experimental.pallas.tpu as pltpu

_RAMP = (1, 1, 2, 2)
_UA, _NA = 4, 7
_U = 20
_NBUF = 3
_NOUT = 2
_NO = 5


def _attention_kernel(q_hbm, k_hbm, v_hbm, o_hbm,
                      q_scr, k_scr, v_scr, o_scr,
                      rq, rk, rv, ro,
                      q01, k0, e_k, e_v, e_o, qt_scr,
                      s00, s01, s10, s11,
                      isem, osem, rsem, asem, xsem, lsem, psem, *, n_heads, scale):
    ramp, UA, NA, U, NBUF, NOUT, NO = _RAMP, _UA, _NA, _U, _NBUF, _NOUT, _NO
    R0 = sum(ramp)
    R = R0 + UA * NA
    NIT = (n_heads - 2 - R) // U
    HU = U // NO
    last = n_heads - 1
    Sq = q_scr.shape[-1]
    Sk = k_scr.shape[-1]
    c = scale * math.log2(math.e)
    q_halves = ((0, 256), (256, Sq))
    k_halves = ((0, Sk // 2), (Sk // 2, Sk))
    s_scr = (s00, s01, s10, s11)
    copy = pltpu.make_async_copy

    def in_copies(it, slot):
        a = R + it * U
        return (
            copy(k_hbm.at[pl.ds(a + 1, U)], k_scr.at[slot], isem.at[slot, 0]),
            copy(v_hbm.at[pl.ds(a, U)], v_scr.at[slot], isem.at[slot, 1]),
            copy(q_hbm.at[pl.ds(a + 2, U)], q_scr.at[slot], isem.at[slot, 2]),
        )

    def out_copy(it, slot, j):
        return copy(o_scr.at[slot, pl.ds(j * HU, HU)],
                    o_hbm.at[pl.ds(R + it * U + j * HU, HU)], osem.at[slot])

    def out_wait(slot):
        copy(o_scr.at[slot], o_scr.at[slot], osem.at[slot]).wait()

    def start_copies(a, n, sem):
        return (
            copy(k_hbm.at[pl.ds(a + 1, n)], rk.at[pl.ds(a, n)], sem.at[0]),
            copy(v_hbm.at[pl.ds(a, n)], rv.at[pl.ds(a, n)], sem.at[1]),
            copy(q_hbm.at[pl.ds(a + 2, n)], rq.at[pl.ds(a, n)], sem.at[2]),
        )

    LP = R // NIT

    def late_out(a, n):
        return copy(ro.at[pl.ds(a, n)], o_hbm.at[pl.ds(a, n)], lsem)

    def ramp_copies(i):
        return start_copies(sum(ramp[:i]), ramp[i], rsem.at[i])

    def a_copies(i):
        return start_copies(R0 + i * UA, UA, asem.at[i])

    k0_copy = copy(k_hbm.at[0], k0, xsem.at[0])
    q01_copy = copy(q_hbm.at[pl.ds(0, 2)], q01, xsem.at[1])
    ek_copy = copy(k_hbm.at[pl.ds(last, 1)], e_k, xsem.at[2])
    ev_copy = copy(v_hbm.at[pl.ds(last - 1, 2)], e_v, xsem.at[3])
    eo_copies = [copy(e_o.at[j], o_hbm.at[last - 1 + j], xsem.at[4 + j]) for j in range(2)]

    def qk(q, kt_ref, par, ia):
        for h, (a, b) in enumerate(k_halves):
            s = jnp.dot(q, kt_ref[:, a:b], preferred_element_type=jnp.float32)
            s_scr[par * 2 + h][ia] = s

    def softmax(par, a, b, ib):
        s0 = s_scr[par * 2 + 0][ib, a:b]
        s1 = s_scr[par * 2 + 1][ib, a:b]
        m = jnp.maximum(jnp.max(s0, axis=1, keepdims=True), jnp.max(s1, axis=1, keepdims=True))
        p0 = jnp.exp2((s0 - m) * c)
        p1 = jnp.exp2((s1 - m) * c)
        l = jnp.sum(p0, axis=1, keepdims=True) + jnp.sum(p1, axis=1, keepdims=True)
        r = pl.reciprocal(l, approx=True)
        r = r * (2.0 - l * r)
        return jnp.concatenate([(p0 * r).astype(jnp.bfloat16),
                                (p1 * r).astype(jnp.bfloat16)], axis=1)

    def pv(vt_ref, o_ref, par, ib):
        ps = [softmax(par, a, b, ib) for a, b in q_halves]
        vt = vt_ref[...]
        for (a, b), p in zip(q_halves, ps):
            ot = lax.dot_general(vt, p, (((1,), (1,)), ((), ())),
                                 preferred_element_type=jnp.float32)
            o_ref[:, a:b] = ot.astype(o_ref.dtype)

    def segment(n, par0, q_ref, k_ref, v_ref, o_ref, ia, ib, hooks, lookahead=True):
        for g in range(n):
            q = qt_scr[...] if g == 0 else q_ref[g - 1].T
            qk(q, k_ref.at[g], (par0 + g + 1) % 2, ia)
            if g == n - 1 and lookahead:
                qt_scr[...] = q_ref[n - 1].T
            pv(v_ref.at[g], o_ref.at[g], (par0 + g) % 2, ib)
            if g in hooks:
                hooks[g]()

    def start_all(copies):
        for cp in copies:
            cp.start()

    groups = [(k0_copy,), (q01_copy,)]
    groups += [ramp_copies(i) for i in range(len(ramp))]
    groups += [a_copies(i) for i in range(NA)]
    groups += [in_copies(j, j) for j in range(NBUF - 1)]
    groups += [(ek_copy, ev_copy)]
    for grp in groups:
        start_all(grp)
        pl.semaphore_signal(psem, 1)
        pl.semaphore_wait(psem, 1)

    k0_copy.wait()
    q01_copy.wait()
    qk(q01[0].T, k0, 0, 0)
    qt_scr[...] = q01[1].T
    for i, n in enumerate(ramp):
        a = sum(ramp[:i])
        for cp in ramp_copies(i):
            cp.wait()
        segment(n, a % 2, rq.at[pl.ds(a, n)], rk.at[pl.ds(a, n)], rv.at[pl.ds(a, n)],
                ro.at[pl.ds(a, n)], 0, 0, {})

    def body_a(i, zero):
        for cp in a_copies(i):
            cp.wait()
        a = R0 + i * UA
        segment(UA, R0 % 2, rq.at[pl.ds(a, UA)], rk.at[pl.ds(a, UA)], rv.at[pl.ds(a, UA)],
                ro.at[pl.ds(a, UA)], i // NA, zero, {})
        return zero

    lax.fori_loop(0, NA, body_a, 0)

    def body(it, carry):
        zero, slot = carry
        nslot = jnp.where(slot == 0, NBUF - 1, slot - 1)
        oslot = lax.rem(it, NOUT)

        @pl.when(it + (NBUF - 1) < NIT)
        def _():
            start_all(in_copies(it + (NBUF - 1), nslot))

        @pl.when(it >= NOUT)
        def _():
            out_wait(oslot)

        for cp in in_copies(it, slot):
            cp.wait()

        hooks = {HU * (j + 1) - 1: functools.partial(lambda j: out_copy(it, oslot, j).start(), j)
                 for j in range(NO)}
        assert 0 not in hooks
        hooks[0] = lambda: late_out(it * LP, LP).start()
        segment(U, R % 2, q_scr.at[slot], k_scr.at[slot], v_scr.at[slot], o_scr.at[oslot],
                it // NIT, zero, hooks)
        return zero, jnp.where(slot == NBUF - 1, 0, slot + 1)

    lax.fori_loop(0, NIT, body, (jnp.int32(0), jnp.int32(0)))

    if R > LP * NIT:
        late_out(LP * NIT, R - LP * NIT).start()
    ek_copy.wait()
    ev_copy.wait()
    segment(1, last % 2 ^ 1, None, e_k, e_v, e_o, 0, 0, {0: eo_copies[0].start}, lookahead=False)
    pv(e_v.at[1], e_o.at[1], last % 2, 0)
    eo_copies[1].start()
    for slot in range(NOUT):
        out_wait(slot)
    late_out(0, R).wait()
    for cp in eo_copies:
        cp.wait()


@jax.jit
def pallas_standalone__mha_softmax__near_ridge_kernel(
    q: jax.Array,
    k: jax.Array,
    v: jax.Array,
):
    B, H, Sq, D = q.shape
    Sk = k.shape[2]
    n_heads = B * H
    ramp, UA, NA, U, NBUF, NOUT, NO = _RAMP, _UA, _NA, _U, _NBUF, _NOUT, _NO
    R = sum(ramp) + UA * NA
    NIT = (n_heads - 2 - R) // U
    assert R + NIT * U + 2 == n_heads and NIT > max(NA, NOUT) and NIT >= NBUF
    assert U % 2 == 0 and UA % 2 == 0 and U % NO == 0
    assert Sk % 256 == 0 and 256 < Sq <= 512

    qt = jnp.swapaxes(q, 2, 3).reshape(n_heads, D, Sq)
    kt = jnp.swapaxes(k, 2, 3).reshape(n_heads, D, Sk)
    vt = jnp.swapaxes(v, 2, 3).reshape(n_heads, D, Sk)

    dt = q.dtype
    vmem, dma = pltpu.VMEM, pltpu.SemaphoreType.DMA
    scratch = [
        vmem((NBUF, U, D, Sq), dt), vmem((NBUF, U, D, Sk), dt), vmem((NBUF, U, D, Sk), dt),
        vmem((NOUT, U, D, Sq), dt),
        vmem((R, D, Sq), dt), vmem((R, D, Sk), dt), vmem((R, D, Sk), dt), vmem((R, D, Sq), dt),
        vmem((2, D, Sq), dt), vmem((D, Sk), dt), vmem((1, D, Sk), dt), vmem((2, D, Sk), dt),
        vmem((2, D, Sq), dt), vmem((Sq, D), dt),
    ]
    scratch += [vmem((1, Sq, Sk // 2), jnp.float32) for _ in range(4)]
    scratch += [
        dma((NBUF, 3)), dma((NOUT,)), dma((len(ramp), 3)), dma((NA, 3)), dma((6,)), dma,
        pltpu.SemaphoreType.REGULAR,
    ]

    ot = pl.pallas_call(
        functools.partial(_attention_kernel, n_heads=n_heads, scale=D ** -0.5),
        in_specs=[pl.BlockSpec(memory_space=pl.ANY)] * 3,
        out_specs=pl.BlockSpec(memory_space=pl.ANY),
        out_shape=jax.ShapeDtypeStruct((n_heads, D, Sq), dt),
        scratch_shapes=scratch,
        compiler_params=pltpu.CompilerParams(
            vmem_limit_bytes=100 * 1024 * 1024,
            disable_bounds_checks=True,
            disable_semaphore_checks=True),
    )(qt, kt, vt)
    return jnp.swapaxes(ot.reshape(B, H, D, Sq), 2, 3)
```
